```python
import os as _os
_os.environ.setdefault("JAX_PLATFORMS", "cpu")
import jax
import jax.numpy as jnp

def _softmax(x, axis=-1):
    return jax.nn.softmax(x, axis=axis)
def _gelu(x):
    return jax.nn.gelu(x, approximate=True)
def _silu(x):
    return jax.nn.silu(x)
def _sigmoid(x):
    return jax.nn.sigmoid(x)
def _layernorm(x, axis=-1, eps=1e-5):
    m = jnp.mean(x, axis=axis, keepdims=True)
    v = jnp.var(x, axis=axis, keepdims=True)
    return (x - m) / jnp.sqrt(v + eps)
def _scatter_add(tgt, idx, src, axis=0):
    return tgt.at[idx].add(src)
def _segment_sum(src, seg, n):
    return jax.ops.segment_sum(src, seg, n)
class _Rng:
    def __init__(self, key):
        self._k = key
    def _next(self):
        self._k, sub = jax.random.split(self._k)
        return sub
    def normal(self, shape):
        return jax.random.normal(self._next(), shape, dtype=jnp.bfloat16)
    def randint(self, lo, hi, shape):
        return jax.random.randint(self._next(), shape, lo, hi, dtype=jnp.int32)
    def uniform(self, shape, lo=0.0, hi=1.0):
        return jax.random.uniform(self._next(), shape, jnp.bfloat16, lo, hi)
    def permutation(self, n):
        return jax.random.permutation(self._next(), n)


kernel_name = 'sequential_preLN__sliding_local_dilated__dense_activation_silu__prompt'

def setup_inputs():
    _rng = _Rng(jax.random.key(int.from_bytes(__import__("os").urandom(4), "little")))
    _w = (lambda a: (lambda t: t.astype(jnp.bfloat16) if jnp.issubdtype(t.dtype, jnp.floating) else t)(jnp.asarray(a)))
    def _A_setup():
        B, S, D = 1, 2048, 1024
        return {
            "x": _w((lambda *s: _rng.normal(s) * 0.05)(B, S, D)),
            "wqkv": _w((lambda *s: _rng.normal(s) * 0.05)(D, 3 * D)),
            "wo": _w((lambda *s: _rng.normal(s) * 0.05)(D, D)),
        }
    _A_in = _A_setup()

    def _B_setup():
        B, S, D, F = 1, 2048, 1024, 3584
        return {
            "x": _w((lambda *s: _rng.normal(s) * 0.05)(B, S, D)),
            "w1": _w((lambda *s: _rng.normal(s) * 0.05)(D, F) * (D ** -0.5)),
            "w2": _w((lambda *s: _rng.normal(s) * 0.05)(F, D) * (F ** -0.5)),
        }
    _B_in = _B_setup()

    return {
        "A_x": _A_in["x"],
        "A_wqkv": _A_in["wqkv"],
        "A_wo": _A_in["wo"],
        "B_x": _B_in["x"],
        "B_w1": _B_in["w1"],
        "B_w2": _B_in["w2"],
    }

def reference(A_x, A_wqkv, A_wo, B_x, B_w1, B_w2):
    def _A_ref(x, wqkv, wo):
        B, S, D = x.shape
        H = 32; Dh = D // H
        W, dil = 8, 2
        qkv = (lambda x, *d: x.transpose(*d))((x @ wqkv).reshape(B, S, 3, H, Dh), 2, 0, 3, 1, 4)
        q, k, v = qkv[0], qkv[1], qkv[2]
        scale = Dh ** -0.5
        pos = jnp.arange(S)
        off = jnp.arange(W) * dil
        idx = pos[:, None] - off[None, :]
        mask = idx >= 0
        idx_c = jnp.where(mask, idx, 0).reshape(-1)
        kg = k[:, :, idx_c, :].reshape(B, H, S, W, Dh)
        vg = v[:, :, idx_c, :].reshape(B, H, S, W, Dh)
        logits = jnp.einsum("bhsd,bhswd->bhsw", q, kg) * scale
        logits = jnp.where(mask[None, None, :, :], logits, -1e9)
        attn = _softmax(logits, axis=-1)
        o = jnp.einsum("bhsw,bhswd->bhsd", attn, vg)
        return (lambda x, *d: x.transpose(*d))(o, 0, 2, 1, 3).reshape(B, S, D) @ wo

    def _B_ref(x, w1, w2):
        h = jnp.einsum("bsd,df->bsf", x, w1)
        h = _silu(h)
        out = jnp.einsum("bsf,fd->bsd", h, w2)
        return out

    x = A_x
    h = x + _A_ref(_layernorm(x, axis=-1), A_wqkv, A_wo)
    h2 = h + _B_ref(_layernorm(h, axis=-1), B_w1, B_w2)
    return h2
```

```python
import functools, contextlib
import jax, jax.numpy as jnp
from jax import lax
import jax.experimental.pallas as pl
import jax.experimental.pallas.tpu as pltpu

F32, BF16, U32 = jnp.float32, jnp.bfloat16, jnp.uint32
NH, WIN, DIL, EPS = 32, 8, 2, 1e-5
HALO = 16
LOG2E = 1.4426950408889634
GS = 33
TM = 256
HM = TM // 2
NT_DIMS = (((1,), (1,)), ((), ()))
QUADS = ((0, 0), (0, 1), (1, 0), (1, 1))
P = functools.partial


def _split(u):
    return tuple(pltpu.unpack_elementwise(u, index=i, packed_dtype=BF16, unpacked_dtype=F32) for i in range(2))


def _join(even, odd):
    return pltpu.pack_elementwise((even, odd), packed_dtype=BF16)


def _bf16(u):
    return pltpu.bitcast(u, BF16)


def _lhs_ops(a11, a12, a21, a22):
    return (a11 + a22, a21 + a22, a11, a22, a11 + a12, a21 - a11, a12 - a22)


def _rhs_ops(b11, b12, b21, b22):
    return (b11 + b22, b11, b12 - b22, b21 - b11, b22, b11 + b12, b21 + b22)


def _combine(m):
    m1, m2, m3, m4, m5, m6, m7 = m
    return m1 + m4 - m5 + m7, m3 + m5, m2 + m4, m1 - m2 + m3 + m6


def _tree(fn, xs):
    xs = list(xs)
    while len(xs) > 1:
        xs = [fn(*xs[i:i + 2]) if i + 1 < len(xs) else xs[i] for i in range(0, len(xs), 2)]
    return xs[0]


def _interleave(main, *sides):
    slots = [[] for _ in range(len(main) + 1)]
    for thunks, lo, hi in sides:
        for k, t in enumerate(thunks):
            slots[lo + (k * (hi - lo)) // len(thunks)].append(t)
    running = []
    for k in range(len(main) + 1):
        for t in slots[k]:
            g = t()
            if g is not None:
                running.append([0, g])
        for item in list(running):
            if item[0] <= k:
                try:
                    item[0] = k + next(item[1])
                except StopIteration:
                    running.remove(item)
        if k < len(main):
            main[k]()
    while running:
        for item in list(running):
            try:
                next(item[1])
            except StopIteration:
                running.remove(item)


def make(WCH=4, flags=None, cfg=None, lag=None, scopes=False):
    lg = dict(pv=2, prep=2, pr=2, ln=2, s1=2, s2=1, l1=1, l2=1)
    lg.update(lag or {})
    c_ = dict(pv=(2, 54), p1=(2, 28), p2=(28, 56), pr=(58, 108), ln=(86, 108),
              f_pr=(58, 82), ln2=(100, 122), e_ln=(2, 26))
    c_.update(cfg or {})

    def kern(x_hbm, wqkv_hbm, wo_hbm, w1_hbm, w2_hbm, o_hbm,
             x_v, wqkv_v, wo_v, w1_v, w2_v,
             bq_s, bk_s, bv_s, bo_s, b1_s, b2_s,
             xa_s, oa_s, ha_s, a2_s, q_s, k_s, v_s, p_s, h_s, out_s, z_s,
             xsem, wsem, fsem, osem):
        S, D = x_v.shape
        F = w2_v.shape[1] * 2
        NT = S // TM
        NC = D // 128
        HC = NC // 2
        FH = F // 2
        FS = FH // (NT - 1)
        CW = D // WCH
        dh = D // NH
        zero = pl.semaphore_read(z_s).astype(U32)
        done = []

        def after(lag, v):
            if len(done) < lag:
                return v
            if v.shape[1] > 128:
                return jnp.concatenate([after(lag, v[:, :128]), v[:, 128:]], axis=1)
            g = pltpu.bitcast(done[-lag][0:8, :], U32) & zero
            return pltpu.bitcast(pltpu.bitcast(v, U32) | g, v.dtype)

        def scaled(i, s):
            return i * s if isinstance(i, int) else pl.multiple_of(i * s, s)

        def x_copy(i):
            r = scaled(i, TM)
            return pltpu.make_async_copy(x_hbm.at[pl.ds(r, TM)], x_v.at[pl.ds(r, TM)], xsem.at[i])

        def w_copy(m, j):
            if m < 3:
                c = m * D + j * CW
                return pltpu.make_async_copy(wqkv_hbm.at[:, pl.ds(c, CW)], wqkv_v.at[:, pl.ds(c, CW)], wsem.at[m * WCH + j])
            return pltpu.make_async_copy(wo_hbm.at[pl.ds(j * CW, CW)], wo_v.at[pl.ds(j * CW, CW)], wsem.at[m * WCH + j])

        def f_copies(j):
            c = scaled(j, FS)
            out = []
            for half in range(2):
                out.append(pltpu.make_async_copy(w1_hbm.at[:, pl.ds(half * FH + c, FS)], w1_v.at[j, half], fsem.at[j * 4 + half]))
                out.append(pltpu.make_async_copy(w2_hbm.at[pl.ds(half * FH + c, FS)], w2_v.at[half, pl.ds(c, FS)], fsem.at[j * 4 + 2 + half]))
            return out

        def scatter(dst, col, pair, blocks):
            f = [[_split(after(lg["prep"], b) if a == 0 else b) for a, b in enumerate(bq)] for bq in blocks]
            for e in range(2):
                ops = [_rhs_ops(*[f[q][a][e] for q in range(4)]) for a in range(2)]
                for t in range(7):
                    dst[t, col, pl.ds(16 * e + pair, 8, stride=GS), :] = _join(ops[0][t], ops[1][t])

        def prep_qkv(m, g, kt):
            c = m * D + scaled(g, 128)
            tt = [pltpu.bitcast(wqkv_v[(kt + HC * dr) * 128:(kt + HC * dr + 1) * 128, pl.ds(c, 128)].T, U32) for dr in range(2)]
            for hp in range(2):
                scatter((bq_s, bk_s, bv_s)[m], kt, 2 * g + hp,
                        [[tt[dr][32 * hp + 16 * a + 8 * dc:32 * hp + 16 * a + 8 * dc + 8] for a in range(2)] for dr, dc in QUADS])

        def prep_o(g, nt):
            for hp in range(2):
                def ld(a, dr, dc):
                    r = g * 128 + 64 * hp + 32 * a + 16 * dr
                    return pltpu.bitcast(wo_v[r:r + 16, (nt + HC * dc) * 128:(nt + HC * dc + 1) * 128], U32)
                scatter(bo_s, nt, 2 * g + hp, [[ld(a, dr, dc) for a in range(2)] for dr, dc in QUADS])

        def ffn_ops(b):
            b = [after(lg["prep"], b[0]), after(lg["prep"], b[1]), after(lg["prep"], b[2]), b[3]]
            f = [_split(u) for u in b]
            ops = [_rhs_ops(*[f[q][e] for q in range(4)]) for e in range(2)]
            return [b[0] if t == 1 else b[3] if t == 4 else _join(ops[0][t], ops[1][t]) for t in range(7)]

        def prep_w1(j, r, c):
            b = [pltpu.bitcast(w1_v[j, dc, dr * (D // 2) + r:dr * (D // 2) + r + 16, c:c + 128], U32) for dr, dc in QUADS]
            for t, v in enumerate(ffn_ops(b)):
                b1_s[j, t, r // 2:r // 2 + 8, c:c + 128] = v

        def prep_w2(j, r, c):
            rows = pl.ds(scaled(j, FS) + r, 16)
            b = [pltpu.bitcast(w2_v[dr, rows, dc * (D // 2) + c:dc * (D // 2) + c + 128], U32) for dr, dc in QUADS]
            for t, v in enumerate(ffn_ops(b)):
                b2_s[t, pl.ds(scaled(j, FS // 2) + r // 2, 8), c:c + 128] = v

        def perm_rows(ref, t, col, g0, ng):
            return jnp.concatenate([ref[t, col, GS * g:GS * g + 32, :] for g in range(g0, g0 + ng)], axis=0)

        def ln_unit(load, dst, scale, r):
            xs = [after(lg["ln"], t) for rr in (r, r + HM) for t in load(rr)]
            mu = [jnp.broadcast_to(jnp.sum(t, axis=-1, keepdims=True), (8, 128)) for t in xs]
            yield lg["l1"]
            xs = [t - jnp.tile(after(lg["ln"], m) * (1.0 / D), (1, NC)) for t, m in zip(xs, mu)]
            var = [jnp.broadcast_to(jnp.sum(t * t, axis=-1, keepdims=True), (8, 128)) for t in xs]
            yield lg["l2"]
            rs = [lax.rsqrt(after(lg["ln"], v) * (1.0 / D) + EPS) for v in var]
            if scale != 1.0:
                rs = [t * scale for t in rs]
            ys = [t * jnp.tile(s_, (1, NC)) for t, s_ in zip(xs, rs)]
            ops = [_lhs_ops(ys[e][:, :D // 2], ys[e][:, D // 2:], ys[2 + e][:, :D // 2], ys[2 + e][:, D // 2:]) for e in range(2)]
            for t in range(7):
                dst[t, r // 2:r // 2 + 8, :] = _join(ops[0][t], ops[1][t])

        def ln1_units(i, dst):
            r0 = scaled(i, TM)
            load = lambda r: _split(pltpu.bitcast(x_v[pl.ds(r0 + r, 16), :], U32))
            return [P(ln_unit, load, dst, 1.0, r) for r in range(0, HM, 16)]

        def ln2_units(i):
            r0 = scaled(i, TM)
            load = lambda r: [jnp.concatenate([h_s[c, pl.ds(r0 + r + e, 8, stride=2), :] for c in range(NC)], axis=1) for e in range(2)]
            return [P(ln_unit, load, ha_s, 0.5, r) for r in range(0, HM, 16)]

        def strassen(n_chunks, product, finish):
            m = []

            def step(n, t):
                m.append(product(n, t))
                done.append(m[-1])
                if t == 6:
                    finish(n, _combine(m))
                    m.clear()
            return [P(step, n, t) for n in range(n_chunks) for t in range(7)]

        def proj(a_s, b_s, dst, halo):
            def product(n, t):
                rhs = jnp.concatenate([_bf16(perm_rows(b_s, t, kt, 2 * n, 2)) for kt in range(HC)], axis=1)
                return lax.dot_general(_bf16(a_s[t]), rhs, NT_DIMS, preferred_element_type=F32)

            def finish(n, cs):
                for (dr, dc), cv in zip(QUADS, cs):
                    dst[n + dc * HC, halo + dr * HM:halo + (dr + 1) * HM, :] = cv
            return strassen(HC, product, finish)

        row2 = 2 * lax.broadcasted_iota(jnp.int32, (8, 128), 0)

        def probs(first, r, e):
            qv = [q_s[c, pl.ds(r + e, 8, stride=2), :] for c in range(NC)]
            qv[0] = after(lg["pr"], qv[0])
            ts = []
            for w in range(WIN):
                rows = pl.ds(HALO + r + e - DIL * w, 8, stride=2)
                t = qv[0] * k_s[0, rows, :]
                for c in range(1, NC):
                    t = t + qv[c] * k_s[c, rows, :]
                ts.append([t] + [pltpu.roll(t, NH * s_, 1) for s_ in range(1, 128 // NH)])
            ls = [_tree(jnp.add, t) for t in ts]
            if first:
                ls = [jnp.where(row2 + (r + e) >= DIL * w, t, -1e9 * dh ** 0.5) if r + e < DIL * w else t for w, t in enumerate(ls)]
            mx = _tree(jnp.maximum, ls)
            yield lg["s1"]
            mx = after(lg["pr"], mx)
            es = [jnp.exp2((t - mx) * (dh ** -0.5 * LOG2E)) for t in ls]
            sm = _tree(jnp.add, es)
            yield lg["s2"]
            inv = 1.0 / after(lg["pr"], sm)
            for w in range(WIN):
                p_s[w, r + 8 * e:r + 8 * e + 8, :] = es[w] * inv

        def probs_units(first):
            return [P(probs, first, r, e) for r in range(0, TM, 16) for e in range(2)]

        def pv_unit(n, r):
            ops = []
            for e in range(2):
                blk = []
                for rr in (r, r + HM):
                    ps = [p_s[w, rr + 8 * e:rr + 8 * e + 8, :] for w in range(WIN)]
                    ps[0] = after(lg["pv"], ps[0])
                    for c in (n, n + HC):
                        acc = None
                        for w in range(WIN):
                            t = ps[w] * v_s[c, pl.ds(HALO + rr + e - DIL * w, 8, stride=2), :]
                            acc = t if acc is None else acc + t
                        blk.append(acc)
                ops.append(_lhs_ops(*blk))
                if e == 0:
                    yield 1
            for t in range(7):
                oa_s[t, r // 2:r // 2 + 8, n * 128:(n + 1) * 128] = _join(ops[0][t], ops[1][t])

        def pv_units():
            return [P(pv_unit, n, r) for n in range(HC) for r in range(0, HM, 16)]

        def out_proj(i):
            r0 = scaled(i, TM)

            def product(n, t):
                return jnp.dot(_bf16(oa_s[t]), _bf16(perm_rows(bo_s, t, n, 0, 8)), preferred_element_type=F32)

            def finish(n, cs):
                for (dr, dc), cv in zip(QUADS, cs):
                    rows, c = pl.ds(r0 + dr * HM, HM), n + dc * HC
                    h_s[c, rows, :] = x_v[rows, c * 128:(c + 1) * 128].astype(F32) + cv
            return strassen(HC, product, finish)

        def shift_halo(ref):
            for c in range(NC):
                ref[c, 0:HALO, :] = ref[c, TM:TM + HALO, :]

        sc = jax.named_scope("pro") if scopes else contextlib.nullcontext()
        sc.__enter__()
        x_copy(0).start()
        for j in range(WCH):
            w_copy(0, j).start()
        for c in range(NC):
            k_s[c, 0:HALO, :] = jnp.zeros((HALO, 128), F32)
        x_copy(0).wait()
        _interleave([], (ln1_units(0, oa_s), 0, 0))
        GPC = NC // WCH

        def prep_q_group(g, carry):
            for kt in range(HC):
                prep_qkv(0, g, kt)
            return carry
        for j in range(WCH):
            w_copy(0, j).wait()
            w_copy(1, j).start()
            lax.fori_loop(j * GPC, (j + 1) * GPC, prep_q_group, 0)

        def arrive(m, j):
            w_copy(m, j).wait()
            if m < 3:
                w_copy(m + 1, j).start()
            elif j == 0:
                x_copy(1).start()
                x_copy(2).start()
            elif j == 1:
                for cp in f_copies(0):
                    cp.start()

        def prep_units(m):
            out = []
            for g in range(NC):
                if g % GPC == 0:
                    out.append(P(arrive, m, g // GPC))
                out += [P(prep_qkv, m, g, kt) if m < 3 else P(prep_o, g, kt) for kt in range(HC)]
            return out

        def v_halo():
            for c in range(NC):
                v_s[c, 0:HALO, :] = jnp.broadcast_to(v_s[c, HALO:HALO + 1, :], (HALO, 128))

        sc.__exit__(None, None, None)
        sc = jax.named_scope("first") if scopes else contextlib.nullcontext()
        sc.__enter__()
        _interleave(proj(oa_s, bq_s, q_s, 0) + proj(oa_s, bk_s, k_s, HALO) + proj(oa_s, bv_s, v_s, HALO),
                    (prep_units(1), 2, 28), (prep_units(2), 30, 56), (prep_units(3), 58, 84),
                    (probs_units(True), *c_["f_pr"]))
        done.clear()
        v_halo()
        x_copy(1).wait()
        _interleave([], (ln1_units(1, xa_s), 0, 0))
        x_copy(3).start()
        for cp in f_copies(1):
            cp.start()

        def attn_body(i, carry):
            done.clear()
            for cp in f_copies(i - 1):
                cp.wait()

            @pl.when(i < NT - 1)
            def _():
                x_copy(i + 1).wait()
            shift_halo(k_s)
            _interleave(
                proj(xa_s, bq_s, q_s, 0) + proj(xa_s, bk_s, k_s, HALO) + proj(xa_s, bv_s, v_s, HALO) + out_proj(i - 1),
                (pv_units(), *c_["pv"]), ([P(shift_halo, v_s)], 56, 56),
                ([P(prep_w1, i - 1, r, c) for r in range(0, D // 2, 16) for c in range(0, FS, 128)], *c_["p1"]),
                ([P(prep_w2, i - 1, r, c) for r in range(0, FS, 16) for c in range(0, D // 2, 128)], *c_["p2"]),
                (probs_units(False), *c_["pr"]),
                (ln1_units(jnp.minimum(i + 1, NT - 1), xa_s), *c_["ln"]))

            @pl.when(i < NT - 3)
            def _():
                x_copy(i + 3).start()

            @pl.when(i < NT - 2)
            def _():
                for cp in f_copies(i + 1):
                    cp.start()
            return carry
        sc.__exit__(None, None, None)
        lax.fori_loop(1, NT, jax.named_scope("attn")(attn_body) if scopes else attn_body, 0)
        sc = jax.named_scope("epi") if scopes else contextlib.nullcontext()
        sc.__enter__()

        done.clear()
        _interleave([], (pv_units(), 0, 0))
        _interleave(out_proj(NT - 1))
        done.clear()
        _interleave([], (ln2_units(0), 0, 0))

        def o_copy(i, slot):
            return pltpu.make_async_copy(out_s.at[slot], o_hbm.at[pl.ds(scaled(i, TM), TM)], osem.at[slot])

        def ffn_body(i, carry):
            done.clear()
            slot = i % 2

            @pl.when(i >= 2)
            def _():
                o_copy(i - 2, slot).wait()
            r0 = scaled(i, TM)

            def up(n, t):
                j, c = divmod(n * 128, FS)
                return jnp.dot(_bf16(ha_s[t]), _bf16(b1_s[j, t, :, c:c + 128]), preferred_element_type=F32)

            def act(n, cs):
                for t, v in enumerate(_lhs_ops(*[y + y * jnp.tanh(y) for y in cs])):
                    a2_s[t, :, n * 128:(n + 1) * 128] = pltpu.bitcast(v.astype(BF16), U32)

            def down(n, t):
                return jnp.dot(_bf16(a2_s[t]), _bf16(b2_s[t, :, n * 128:(n + 1) * 128]), preferred_element_type=F32)

            def fin(n, cs):
                for (dr, dc), cv in zip(QUADS, cs):
                    c = n + dc * HC
                    out_s[slot, dr * HM:(dr + 1) * HM, c * 128:(c + 1) * 128] = (h_s[c, pl.ds(r0 + dr * HM, HM), :] + cv).astype(BF16)
            _interleave(strassen(FH // 128, up, act) + strassen(HC, down, fin),
                        (ln2_units(jnp.minimum(i + 1, NT - 1)), *c_["ln2"]))
            o_copy(i, slot).start()
            return carry
        sc.__exit__(None, None, None)
        lax.fori_loop(0, NT, jax.named_scope("ffn")(ffn_body) if scopes else ffn_body, 0)
        for ii in (NT - 2, NT - 1):
            o_copy(ii, ii % 2).wait()

    def fn(A_x, A_wqkv, A_wo, B_x, B_w1, B_w2):
        S, D = A_x.shape[1:]
        F = B_w1.shape[1]
        NT = S // TM
        FS = F // 2 // (NT - 1)
        NC = D // 128
        anyspec = pl.BlockSpec(memory_space=pl.ANY)
        perm = pltpu.VMEM((7, NC // 2, 8 * GS, 128), U32)
        lhs = pltpu.VMEM((7, HM // 2, D // 2), U32)
        out = pl.pallas_call(
            kern,
            in_specs=[anyspec] * 5,
            out_specs=anyspec,
            out_shape=jax.ShapeDtypeStruct((S, D), BF16),
            scratch_shapes=[
                pltpu.VMEM((S, D), BF16), pltpu.VMEM((D, 3 * D), BF16), pltpu.VMEM((D, D), BF16),
                pltpu.VMEM((NT - 1, 2, D, FS), BF16), pltpu.VMEM((2, F // 2, D), BF16),
                perm, perm, perm, perm,
                pltpu.VMEM((NT - 1, 7, D // 4, FS), U32), pltpu.VMEM((7, F // 4, D // 2), U32),
                lhs, lhs, lhs, pltpu.VMEM((7, HM // 2, F // 2), U32),
                pltpu.VMEM((NC, TM, 128), F32), pltpu.VMEM((NC, TM + HALO, 128), F32),
                pltpu.VMEM((NC, TM + HALO, 128), F32), pltpu.VMEM((WIN, TM, 128), F32),
                pltpu.VMEM((NC, S, 128), F32), pltpu.VMEM((2, TM, D), BF16), pltpu.SemaphoreType.REGULAR,
                pltpu.SemaphoreType.DMA((NT,)), pltpu.SemaphoreType.DMA((4 * WCH,)),
                pltpu.SemaphoreType.DMA((4 * (NT - 1),)), pltpu.SemaphoreType.DMA((2,)),
            ],
            compiler_params=pltpu.CompilerParams(vmem_limit_bytes=120 * 1024 * 1024, flags=flags),
        )(A_x.reshape(S, D), A_wqkv, A_wo, B_w1, B_w2)
        return out.reshape(1, S, D)
    return fn


@jax.jit
def pallas_sequential_preLN__sliding_local_dilated__dense_activation_silu__prompt_kernel(
    A_x, A_wqkv, A_wo, B_x, B_w1, B_w2
):
    return make(cfg={'pr':(57,96),'ln':(92,109)})(A_x, A_wqkv, A_wo, B_x, B_w1, B_w2)
```

```python
import functools

import jax
import jax.numpy as jnp
from jax import lax
import jax.experimental.pallas as pl
import jax.experimental.pallas.tpu as pltpu

F32, BF16, U32 = jnp.float32, jnp.bfloat16, jnp.uint32
HEADS, WINDOW, DILATION, EPS = 32, 8, 2, 1e-5
LOG2E = 1.4426950408889634
TM = 256
HM = TM // 2
QM = TM // 4
HALO = 16
GS = 33
NT_DIMS = (((1,), (1,)), ((), ()))
QUADS = ((0, 0), (0, 1), (1, 0), (1, 1))
P = functools.partial


def _split(u):
    return tuple(pltpu.unpack_elementwise(u, index=i, packed_dtype=BF16, unpacked_dtype=F32) for i in range(2))


def _join(even, odd):
    return pltpu.pack_elementwise((even, odd), packed_dtype=BF16)


def _bf16(u):
    return pltpu.bitcast(u, BF16)


def _lhs_ops(a11, a12, a21, a22):
    return (a11 + a22, a21 + a22, a11, a22, a11 + a12, a21 - a11, a12 - a22)


def _rhs_ops(b11, b12, b21, b22):
    return (b11 + b22, b11, b12 - b22, b21 - b11, b22, b11 + b12, b21 + b22)


FEEDS = (((0, 1), (3, 1)), ((2, 1), (3, -1)), ((1, 1), (3, 1)), ((0, 1), (2, 1)),
         ((0, -1), (1, 1)), ((3, 1),), ((0, 1),))
IN_ORDER = (0, 1, 2, 3, 4, 5, 6)
EARLY = (1, 3, 4, 2, 0, 5, 6)
LHS_FETCH = ((0, (2,)), (1, (4,)), (3, (0, 6, 3)), (2, (5, 1)))
RHS_FETCH = ((0, (1,)), (2, (3,)), (3, (0, 6, 4)), (1, (5, 2)))


class _Combine:
    def __init__(self, order, emit):
        self.order, self.emit, self.acc, self.k = order, emit, {}, 0
        self.last = {q: k for k, t in enumerate(order) for q, _ in FEEDS[t]}

    def push(self, m):
        for q, sign in FEEDS[self.order[self.k]]:
            if q not in self.acc:
                self.acc[q] = (sign, m)
            else:
                s, v = self.acc[q]
                self.acc[q] = (s, v + m) if s == sign else (1, v - m) if s > 0 else (1, m - v)
            if self.last[q] == self.k:
                self.emit(q, self.acc.pop(q)[1])
        self.k = (self.k + 1) % 7


class _Absent:
    __add__ = __radd__ = __sub__ = __rsub__ = lambda self, other: self


def _block_index(outer, inner):
    return 2 * (outer // 2) + inner // 2, 2 * (outer % 2) + inner % 2


def _tree(fn, xs):
    xs = list(xs)
    while len(xs) > 1:
        xs = [fn(*xs[i:i + 2]) if i + 1 < len(xs) else xs[i] for i in range(0, len(xs), 2)]
    return xs[0]


def _aligned(i, n):
    return i if isinstance(i, int) else pl.multiple_of(i, n)


def _scaled(i, n):
    return _aligned(i * n, n)


def _start(copies):
    for cp in copies:
        cp.start()


def _wait(copies):
    for cp in copies:
        cp.wait()


class _Schedule:
    def __init__(self):
        self.done = []
        self.slot = 0
        self.zero = None

    def after(self, lag, v):
        if v.shape[1] > 128:
            return jnp.concatenate([self.after(lag, v[:, :128]), v[:, 128:]], axis=1)
        back = max(1, lag - self.slot)
        for m, slots in reversed(self.done):
            if back <= slots:
                r = (slots - back) * m.shape[0] // slots // 16 * 16
                gate = pltpu.bitcast(m[r:r + 8, :], U32) & self.zero
                return pltpu.bitcast(pltpu.bitcast(v, U32) | gate, v.dtype)
            back -= slots
        return v

    def run(self, steps, *sides):
        edge = [0]
        for _, slots in steps:
            edge.append(edge[-1] + slots)
        starts = {}
        for units, lo, hi in sides:
            assert 0 <= lo <= hi <= len(steps)
            for k, unit in enumerate(units):
                starts.setdefault(edge[lo] + k * (edge[hi] - edge[lo]) // len(units), []).append(unit)
        running, step = [], 0
        for k in range(edge[-1] + 1):
            self.slot = k - edge[step]
            for unit in starts.get(k, ()):
                gen = unit()
                if gen is not None:
                    running.append([0, gen])
            for item in list(running):
                if item[0] <= k:
                    try:
                        item[0] = k + next(item[1])
                    except StopIteration:
                        running.remove(item)
            if step < len(steps) and k + 1 == edge[step + 1]:
                steps[step][0]()
                step += 1
        for item in running:
            for _ in item[1]:
                pass


def _kernel(x_hbm, wqkv_hbm, wo_hbm, w1_hbm, w2_hbm, o_hbm,
            stage, w1_v, w2_v,
            bq_s, bk_s, bv_s, bo_s, b1_s, b2_s,
            ox_s, xb_s, ha_s, a2_s,
            q_s, k_s, v_s, p_s, st_s, h_s, out_s,
            xsem, qsem, wsem, fsem, osem):
    S, D = x_hbm.shape
    F = w2_hbm.shape[0]
    NT = S // TM
    NC = D // 128
    HC = NC // 2
    DQ, FQ = D // 4, F // 4
    NF = FQ // 128
    R1, R2 = w1_v.shape[0] - D, w2_v.shape[0] - F
    head_dim = D // HEADS
    oa_s, xa_s = ox_s.at[0], ox_s.at[1]
    sched = _Schedule()
    after, run = sched.after, sched.run

    def x_copy(k):
        rows = pl.ds(k * TM, TM if k < 4 else S - 4 * TM)
        return [pltpu.make_async_copy(x_hbm.at[rows], stage.at[rows], xsem.at[k])]

    def q_copy(g):
        rows = [_scaled(g + HC * half, 128) for half in range(2)]
        return [pltpu.make_async_copy(wqkv_hbm.at[pl.ds(r, 128), pl.ds(0, D)],
                                      stage.at[pl.ds(_aligned(S + r, 128), 128)], qsem.at[g]) for r in rows]

    def w_copy(m):
        src = wo_hbm if m == 3 else wqkv_hbm.at[:, pl.ds(m * D, D)]
        return [pltpu.make_async_copy(src, stage.at[pl.ds(S + m * D, D)], wsem.at[m - 1])]

    def f_copy(g):
        out = []
        for hbm, dst, blk, r in ((w1_hbm, w1_v, DQ, R1), (w2_hbm, w2_v, FQ, R2)):
            for q in range(4):
                rows = pl.ds(q * blk + 2 * r, blk - 2 * r) if g else pl.ds(q * blk, 2 * r)
                out.append(pltpu.make_async_copy(hbm.at[rows], dst.at[rows], fsem.at[g]))
        return out

    def o_copy(i, r0=0, nr=TM, c0=0, nc=D):
        return [pltpu.make_async_copy(out_s.at[i % 2, pl.ds(r0, nr), pl.ds(c0, nc)],
                                      o_hbm.at[pl.ds(_aligned(i * TM + r0, HM), nr), pl.ds(c0, nc)], osem.at[i % 2])]

    def scatter(dst, col, pair, blocks):
        f = []
        for q in range(4):
            f.append([_split(after(12, b)) for b in blocks[q]])
            yield 1
        for e in range(2):
            ops = [_rhs_ops(*[f[q][a][e] for q in range(4)]) for a in range(2)]
            for t in range(7):
                dst[t, col, pl.ds(16 * e + pair, 8, stride=GS), :] = _join(ops[0][t], ops[1][t])

    def prep_qkv(m, g, kt, src=None):
        rows = [_aligned(S + (m if src is None else src) * D + (kt + HC * half) * 128, 128) for half in range(2)]
        tt = [pltpu.bitcast(stage[pl.ds(r, 128), g * 128:(g + 1) * 128].T, U32) for r in rows]
        yield 6
        for hp in range(2):
            yield from scatter((bq_s, bk_s, bv_s)[m], kt, 2 * g + hp,
                               [[tt[dr][32 * hp + 16 * a + 8 * dc:32 * hp + 16 * a + 8 * dc + 8] for a in range(2)]
                                for dr, dc in QUADS])

    def prep_o(pair, nt):
        def load(a, dr, dc):
            r, c = S + 3 * D + 64 * pair + 32 * a + 16 * dr, (nt + HC * dc) * 128
            return pltpu.bitcast(stage[r:r + 16, c:c + 128], U32)
        return scatter(bo_s, nt, pair, [[load(a, dr, dc) for a in range(2)] for dr, dc in QUADS])

    def prep_units(m, src=None):
        if m == 3:
            return [P(prep_o, pair, nt) for pair in range(HEADS // 2) for nt in range(HC)]
        return [P(prep_qkv, m, g, kt, src) for kt in range(HC) for g in range(NC)]

    def two_levels(ops, fetch, pause, load, store):
        f = {}
        for qo, ts in fetch:
            f[qo] = {}
            for qi in (0, 3, 1, 2):
                f[qo][qi] = load(*_block_index(qo, qi))
                yield pause[len(ts) - 1]
            for t in ts:
                outer = [[ops(*[f[q][qi][e] if q in f else _Absent() for q in range(4)])[t] for qi in range(4)]
                         for e in range(2)]
                inner = [ops(*outer[e]) for e in range(2)]
                for u in range(7):
                    store(7 * t + u, _join(inner[0][u], inner[1][u]))

    def prep_ffn(src, dst, col, src_row, src_step, dst_row, r, n):
        def load(rb, cb):
            rows, c = pl.ds(_aligned(src_row + rb * src_step + r, 16), 16), col(cb, n) * 128
            return _split(after(12, pltpu.bitcast(src[rows, c:c + 128], U32)))

        def store(k, v):
            dst[n, k, pl.ds(_aligned(dst_row + r // 2, 8), 8), :] = v
        return two_levels(_rhs_ops, RHS_FETCH, (1, 1, 1), load, store)

    def prep_ffn_units(i):
        out = []
        for src, dst, blk, rows, chunks, col in ((w1_v, b1_s, DQ, R1, NF, lambda cb, n: cb * NF + n),
                                                 (w2_v, b2_s, FQ, R2, 2, lambda cb, n: 4 * n + cb)):
            if isinstance(i, int):
                r0 = (i - 2) * rows
                where, rows = (r0, blk, r0 // 2), blk - r0
            else:
                r0 = jnp.where(i > 1, (i - 2) * rows, 0)
                where = (jnp.where(i > 1, r0, 4 * blk), jnp.where(i > 1, blk, 0), r0 // 2)
            out.append([P(prep_ffn, src, dst, col, *where, r, n) for r in range(0, rows, 16) for n in range(chunks)])
        return out

    def permuted(ref, t, col, g0, groups):
        return jnp.concatenate([ref[t, col, GS * g:GS * g + 32, :] for g in range(g0, g0 + groups)], axis=0)

    def ln_stats(load, scale, r):
        xs = [load(r, c) for c in range(NC)]
        xs = [[after(12, t[e]) if c == 0 else t[e] for c, t in enumerate(xs)] for e in range(2)]
        mu = [jnp.broadcast_to(jnp.sum(_tree(jnp.add, t), axis=-1, keepdims=True), (8, 128)) for t in xs]
        yield 16
        mu = [after(12, m) * (1.0 / D) for m in mu]
        var = [_tree(jnp.add, [(t - m) * (t - m) for t in ts]) for ts, m in zip(xs, mu)]
        var = [jnp.broadcast_to(jnp.sum(v, axis=-1, keepdims=True), (8, 128)) for v in var]
        yield 16
        for e in range(2):
            rs = lax.rsqrt(after(12, var[e]) * (1.0 / D) + EPS)
            st_s[0, r + 8 * e:r + 8 * e + 8, :] = mu[e]
            st_s[1, r + 8 * e:r + 8 * e + 8, :] = rs if scale == 1.0 else rs * scale

    def normalized(load, r, c):
        st = [[st_s[k, r + 8 * e:r + 8 * e + 8, :] for k in range(2)] for e in range(2)]
        return [(t - after(12, m)) * rs for t, (m, rs) in zip(load(r, c), st)]

    def ln_apply(load, dst, r, kt):
        ys = []
        for dr, dc in QUADS:
            ys.append(normalized(load, r + dr * HM, kt + dc * HC))
            yield 1
        ops = [_lhs_ops(*[y[e] for y in ys]) for e in range(2)]
        for t in range(7):
            dst[t, r // 2:r // 2 + 8, kt * 128:(kt + 1) * 128] = _join(ops[0][t], ops[1][t])

    def ln_apply2(load, r, n):
        def store(k, v):
            ha_s[k, r // 2:r // 2 + 8, n * 128:(n + 1) * 128] = v
        return two_levels(_lhs_ops, LHS_FETCH, (1, 2, 2), lambda rb, cb: normalized(load, rb * QM + r, 2 * cb + n), store)

    def ln_x(i, dst):
        r0 = _scaled(i, TM)

        def load(r, c):
            return _split(pltpu.bitcast(stage[pl.ds(r0 + r, 16), c * 128:(c + 1) * 128], U32))
        return ([P(ln_stats, load, 1.0, r) for r in range(0, TM, 16)],
                [P(ln_apply, load, dst, r, kt) for kt in range(HC) for r in range(0, HM, 16)])

    def ln_h(i):
        r0 = _scaled(i, TM)

        def load(r, c):
            return [h_s[c, pl.ds(r0 + r + e, 8, stride=2), :] for e in range(2)]
        return ([P(ln_stats, load, 0.5, r) for r in range(0, TM, 16)],
                [P(ln_apply2, load, r, n) for n in range(2) for r in range(0, QM, 16)])

    def strassen(product, emit):
        steps = []
        for n in range(HC):
            comb = _Combine(EARLY, P(emit, n))

            def step(t, n=n, comb=comb):
                sched.done.append((product(n, t), HM // 16))
                comb.push(sched.done[-1][0])
            steps += [(P(step, t), HM // 16) for t in EARLY]
        return steps

    def strassen2(chunks, k_tiles, product, emit, order):
        steps = []
        for n in range(chunks):
            outer = [_Combine(order, P(emit, n, qi)) for qi in range(4)]
            inner = _Combine(IN_ORDER, lambda qi, c, outer=outer: outer[qi].push(c))

            def step(k, n=n, inner=inner):
                sched.done.append((product(n, k), k_tiles))
                inner.push(sched.done[-1][0])
            steps += [(P(step, 7 * t + u), k_tiles) for t in order for u in IN_ORDER]
        return steps

    def project(a_s, b_s, dst, row):
        def product(n, t):
            rhs = jnp.concatenate([_bf16(permuted(b_s, t, kt, 2 * n, 2)) for kt in range(HC)], axis=1)
            return lax.dot_general(_bf16(a_s[t]), rhs, NT_DIMS, preferred_element_type=F32)

        def emit(n, q, c):
            dr, dc = QUADS[q]
            dst[n + dc * HC, pl.ds(_aligned(row + dr * HM, 8), HM), :] = c
        return strassen(product, emit)

    def out_project(i, a_s):
        r0 = _scaled(i, TM)

        def product(n, t):
            return jnp.dot(_bf16(a_s[t]), _bf16(permuted(bo_s, t, n, 0, NC)), preferred_element_type=F32)

        def emit(n, q, c):
            dr, dc = QUADS[q]
            rows, col = pl.ds(r0 + dr * HM, HM), n + dc * HC
            h_s[col, rows, :] = stage[rows, col * 128:(col + 1) * 128].astype(F32) + c
        return strassen(product, emit)

    row2 = 2 * lax.broadcasted_iota(jnp.int32, (8, 128), 0)

    def probs(first, r, e):
        pause = (0, 6, 4) if first else (2, 8, 6)
        qv = [q_s[c, pl.ds((0 if first else TM) + r + e, 8, stride=2), :] for c in range(NC)]
        ls = []
        for w in range(WINDOW):
            rows = pl.ds(HALO + r + e - DILATION * w, 8, stride=2)
            t = qv[0] * after(16, k_s[0, rows, :])
            for c in range(1, NC):
                t = t + qv[c] * k_s[c, rows, :]
            t = _tree(jnp.add, [t] + [pltpu.roll(t, HEADS * s, 1) for s in range(1, 128 // HEADS)])
            if first and r + e < DILATION * w:
                t = jnp.where(row2 + (r + e) >= DILATION * w, t, -1e9 * head_dim ** 0.5)
            ls.append(t)
            yield pause[0]
        mx = _tree(jnp.maximum, ls)
        yield pause[1]
        mx = after(16, mx)
        es = [jnp.exp2((t - mx) * (head_dim ** -0.5 * LOG2E)) for t in ls]
        total = _tree(jnp.add, es)
        yield pause[2]
        inv = 1.0 / after(16, total)
        for w in range(WINDOW):
            p_s[w, r + 8 * e:r + 8 * e + 8, :] = es[w] * inv

    def probs_units(first):
        return [P(probs, first, r, e) for r in range(0, TM, 16) for e in range(2)]

    def mix(dst, n, r):
        ops = []
        for e in range(2):
            blocks = []
            for rr in (r, r + HM):
                ps = [p_s[w, rr + 8 * e:rr + 8 * e + 8, :] for w in range(WINDOW)]
                for c in (n, n + HC):
                    acc = None
                    for w in range(WINDOW):
                        v = v_s[c, pl.ds(HALO + rr + e - DILATION * w, 8, stride=2), :]
                        acc = ps[w] * after(12, v) if w == 0 else acc + ps[w] * v
                    blocks.append(acc)
                    yield 1
            ops.append(_lhs_ops(*blocks))
        for t in range(7):
            dst[t, r // 2:r // 2 + 8, n * 128:(n + 1) * 128] = _join(ops[0][t], ops[1][t])

    def mix_units(dst):
        return [P(mix, dst, n, r) for n in range(HC) for r in range(0, HM, 16)]

    def shift_halo(ref):
        for c in range(NC):
            ref[c, 0:HALO, :] = ref[c, TM:TM + HALO, :]

    _start(x_copy(0) + x_copy(1) + sum(map(q_copy, range(HC)), []) + w_copy(1) + x_copy(2)
           + w_copy(2) + w_copy(3) + x_copy(3))
    for c in range(NC):
        k_s[c, 0:HALO, :] = jnp.zeros((HALO, 128), F32)
    w1_v[D:, :] = jnp.zeros((R1, F), BF16)
    w2_v[F:, :] = jnp.zeros((R2, D), BF16)
    _wait(x_copy(0))
    word = pltpu.bitcast(stage[0:16, 0:128], U32)
    sched.zero = (word * word) & 2
    _start(f_copy(0))

    def normalize_tile(i, carry):
        pl.when(i == 1)(P(_wait, x_copy(1)))
        for units in ln_x(i, ox_s.at[i]):
            run([], (units, 0, 0))
        return carry
    lax.fori_loop(0, 2, normalize_tile, 0)

    def prepare_q(kt, carry):
        _wait(q_copy(kt))
        run([], ([P(prep_qkv, 0, g, kt) for g in range(NC)], 0, 0))
        return carry
    lax.fori_loop(0, HC, prepare_q, 0)

    def first_q(i, carry):
        sched.done.clear()
        pl.when(i == 1)(P(_wait, w_copy(1)))
        run(project(ox_s.at[i], bq_s, q_s, i * TM), (prep_units(1, i), 1, 27))
        return carry
    lax.fori_loop(0, 2, first_q, 0)

    sched.done.clear()
    _wait(x_copy(2))
    stats, apply = ln_x(2, xb_s)
    run(project(oa_s, bk_s, k_s, HALO) + project(oa_s, bv_s, v_s, HALO),
        (stats, 0, 6), (apply, 8, 27),
        ([P(_wait, w_copy(2)), P(_start, x_copy(4))], 9, 9), (prep_units(2), 9, 27),
        (probs_units(True), 29, 47),
        ([P(_wait, w_copy(3)), P(_start, f_copy(1))], 47, 47), (prep_units(3), 47, 56))
    for c in range(NC):
        v_s[c, 0:HALO, :] = jnp.broadcast_to(v_s[c, HALO:HALO + 1, :], (HALO, 128))

    def move(t, kt):
        xa_s[t, :, kt * 128:(kt + 1) * 128] = xb_s[t, :, kt * 128:(kt + 1) * 128]

    def attention(i, carry):
        sched.done.clear()
        for k, copies in ((1, x_copy(3)), (2, x_copy(4) + f_copy(0)), (4, f_copy(1))):
            pl.when(i == k)(P(_wait, copies))
        shift_halo(k_s)
        prep1, prep2 = prep_ffn_units(i)
        stats, apply = ln_x(jnp.minimum(i + 2, NT - 1), xb_s)
        run(project(xa_s, bk_s, k_s, HALO) + project(xa_s, bv_s, v_s, HALO) + project(xb_s, bq_s, q_s, TM)
            + out_project(i - 1, oa_s),
            (mix_units(oa_s), 1, 27), ([P(shift_halo, v_s)], 28, 28), (probs_units(False), 29, 58),
            ([P(move, t, kt) for t in EARLY for kt in range(HC)], 58, 80),
            (prep1, 58, 84), (prep2, 84, 108), (stats, 60, 82), (apply, 86, 110))
        return carry
    lax.fori_loop(1, NT - 1, attention, 0)

    sched.done.clear()
    shift_halo(k_s)
    prep1, prep2 = prep_ffn_units(NT - 1)
    stats, apply = ln_h(0)
    run(project(xa_s, bk_s, k_s, HALO) + project(xa_s, bv_s, v_s, HALO)
        + out_project(NT - 2, oa_s) + out_project(NT - 1, xb_s),
        (mix_units(oa_s), 1, 26), ([P(shift_halo, v_s)], 28, 28), (probs_units(False), 29, 56),
        (mix_units(xb_s), 60, 82), (prep1, 30, 80), (prep2, 80, 108), (stats, 84, 96), (apply, 98, 110))

    def feed_forward(i, carry):
        sched.done.clear()
        pl.when(i > 1)(lambda: _wait(o_copy(i - 2)))
        r0 = _scaled(i, TM)
        acts = {}

        def up(n, k):
            return jnp.dot(_bf16(ha_s[k]), _bf16(b1_s[n, k]), preferred_element_type=F32)

        def activate(n, qi, qo, y):
            acts[qo, qi] = y + y * jnp.tanh(y)
            if len(acts) == 16:
                outer = [_lhs_ops(*[acts[qo, qi] for qo in range(4)]) for qi in range(4)]
                for t in range(7):
                    for u, v in enumerate(_lhs_ops(*[outer[qi][t] for qi in range(4)])):
                        a2_s[7 * t + u, :, n * 128:(n + 1) * 128] = pltpu.bitcast(v.astype(BF16), U32)
                acts.clear()

        def down(n, k):
            return jnp.dot(_bf16(a2_s[k]), _bf16(b2_s[n, k]), preferred_element_type=F32)

        def finish(n, qi, qo, c):
            rb, cb = _block_index(qo, qi)
            col = 4 * n + cb
            out_s[i % 2, rb * QM:(rb + 1) * QM, col * 128:(col + 1) * 128] = (
                h_s[col, pl.ds(r0 + rb * QM, QM), :] + c).astype(BF16)

        stats, apply = ln_h(jnp.minimum(i + 1, NT - 1))
        last = 49 * (NF + 1)
        run(strassen2(NF, 2, up, activate, EARLY) + strassen2(2, NF, down, finish, IN_ORDER),
            (stats, last + 1, last + 16), (apply, last + 19, last + 45),
            ([P(_start, o_copy(i, 0, TM, 0, D // 2))], last, last),
            ([P(_start, o_copy(i, HM, HM, D // 2, D // 2))], last + 42, last + 42))
        _start(o_copy(i, 0, HM, D // 2, D // 2))
        return carry
    lax.fori_loop(0, NT, feed_forward, 0)
    _wait(o_copy(NT - 2) + o_copy(NT - 1))


@jax.jit
def pallas_sequential_preLN__sliding_local_dilated__dense_activation_silu__prompt_kernel(
    A_x: jax.Array,
    A_wqkv: jax.Array,
    A_wo: jax.Array,
    B_x: jax.Array,
    B_w1: jax.Array,
    B_w2: jax.Array,
):
    del B_x
    B, S, D = A_x.shape
    F = B_w1.shape[1]
    assert (B, S, D, F) == (1, 2048, 1024, 3584)
    NC, slices = D // 128, S // TM - 2
    r1, r2 = (pl.cdiv(n // 4, 16 * slices) * 16 for n in (D, F))
    hbm = pl.BlockSpec(memory_space=pl.ANY)
    projection = pltpu.VMEM((7, NC // 2, 8 * GS, 128), U32)
    out = pl.pallas_call(
        _kernel,
        in_specs=[hbm] * 5,
        out_specs=hbm,
        out_shape=jax.ShapeDtypeStruct((S, D), BF16),
        scratch_shapes=[
            pltpu.VMEM((S + 4 * D, D), BF16), pltpu.VMEM((D + r1, F), BF16), pltpu.VMEM((F + r2, D), BF16),
            projection, projection, projection, projection,
            pltpu.VMEM((F // 512, 49, D // 8, 128), U32), pltpu.VMEM((D // 512, 49, F // 8, 128), U32),
            pltpu.VMEM((2, 7, HM // 2, D // 2), U32), pltpu.VMEM((7, HM // 2, D // 2), U32),
            pltpu.VMEM((49, QM // 2, D // 4), U32), pltpu.VMEM((49, QM // 2, F // 4), U32),
            pltpu.VMEM((NC, 2 * TM, 128), F32), pltpu.VMEM((NC, TM + HALO, 128), F32),
            pltpu.VMEM((NC, TM + HALO, 128), F32), pltpu.VMEM((WINDOW, TM, 128), F32),
            pltpu.VMEM((2, TM, 128), F32), pltpu.VMEM((NC, S, 128), F32), pltpu.VMEM((2, TM, D), BF16),
            pltpu.SemaphoreType.DMA((5,)), pltpu.SemaphoreType.DMA((NC // 2,)), pltpu.SemaphoreType.DMA((3,)),
            pltpu.SemaphoreType.DMA((2,)), pltpu.SemaphoreType.DMA((2,)),
        ],
        compiler_params=pltpu.CompilerParams(vmem_limit_bytes=124 * 1024 * 1024, disable_bounds_checks=True),
    )(A_x.reshape(S, D), A_wqkv, A_wo, B_w1, B_w2)
    return out.reshape(B, S, D)
```

```python
import functools

import jax
import jax.numpy as jnp
from jax import lax
import jax.experimental.pallas as pl
import jax.experimental.pallas.tpu as pltpu

F32, BF16, U32 = jnp.float32, jnp.bfloat16, jnp.uint32
HEADS, WINDOW, DILATION, EPS = 32, 8, 2, 1e-5
LOG2E = 1.4426950408889634
TM = 256
HM = TM // 2
QM = TM // 4
HALO = 16
GS = 33
NT_DIMS = (((1,), (1,)), ((), ()))
QUADS = ((0, 0), (0, 1), (1, 0), (1, 1))
P = functools.partial


def _split(u):
    return tuple(pltpu.unpack_elementwise(u, index=i, packed_dtype=BF16, unpacked_dtype=F32) for i in range(2))


def _join(even, odd):
    return pltpu.pack_elementwise((even, odd), packed_dtype=BF16)


def _bf16(u):
    return pltpu.bitcast(u, BF16)


def _lhs_ops(a11, a12, a21, a22):
    return (a11 + a22, a21 + a22, a11, a22, a11 + a12, a21 - a11, a12 - a22)


def _rhs_ops(b11, b12, b21, b22):
    return (b11 + b22, b11, b12 - b22, b21 - b11, b22, b11 + b12, b21 + b22)


FEEDS = (((0, 1), (3, 1)), ((2, 1), (3, -1)), ((1, 1), (3, 1)), ((0, 1), (2, 1)),
         ((0, -1), (1, 1)), ((3, 1),), ((0, 1),))
EARLY = (1, 3, 4, 2, 0, 5, 6)
LHS_FETCH = ((0, (2,)), (1, (4,)), (3, (0, 6, 3)), (2, (5, 1)))
RHS_FETCH = ((0, (1,)), (2, (3,)), (3, (0, 6, 4)), (1, (5, 2)))


class _Combine:
    def __init__(self, order, emit):
        self.order, self.emit, self.acc, self.k = order, emit, {}, 0
        self.last = {q: k for k, t in enumerate(order) for q, _ in FEEDS[t]}

    def push(self, m):
        for q, sign in FEEDS[self.order[self.k]]:
            if q not in self.acc:
                self.acc[q] = (sign, m)
            else:
                s, v = self.acc[q]
                self.acc[q] = (s, v + m) if s == sign else (1, v - m) if s > 0 else (1, m - v)
            if self.last[q] == self.k:
                self.emit(q, self.acc.pop(q)[1])
        self.k = (self.k + 1) % 7


class _Absent:
    __add__ = __radd__ = __sub__ = __rsub__ = lambda self, other: self


def _block_index(outer, inner):
    return 2 * (outer // 2) + inner // 2, 2 * (outer % 2) + inner % 2


def _tree(fn, xs):
    xs = list(xs)
    while len(xs) > 1:
        xs = [fn(*xs[i:i + 2]) if i + 1 < len(xs) else xs[i] for i in range(0, len(xs), 2)]
    return xs[0]


def _aligned(i, n):
    return i if isinstance(i, int) else pl.multiple_of(i, n)


def _scaled(i, n):
    return _aligned(i * n, n)


def _start(copies):
    for cp in copies:
        cp.start()


def _wait(copies):
    for cp in copies:
        cp.wait()


class _Schedule:
    def __init__(self):
        self.done = []
        self.slot = 0
        self.zero = None

    def after(self, lag, v):
        if v.shape[1] > 128:
            return jnp.concatenate([self.after(lag, v[:, :128]), v[:, 128:]], axis=1)
        back = max(1, lag - self.slot)
        for m, slots in reversed(self.done):
            if back <= slots:
                r = (slots - back) * m.shape[0] // slots // 16 * 16
                gate = pltpu.bitcast(m[r:r + 8, :], U32) & self.zero
                return pltpu.bitcast(pltpu.bitcast(v, U32) | gate, v.dtype)
            back -= slots
        return v

    def run(self, steps, *sides):
        edge = [0]
        for _, slots in steps:
            edge.append(edge[-1] + slots)
        starts = {}
        for units, lo, hi in sides:
            assert 0 <= lo <= hi <= len(steps)
            for k, unit in enumerate(units):
                starts.setdefault(edge[lo] + k * (edge[hi] - edge[lo]) // len(units), []).append(unit)
        running, step = [], 0
        for k in range(edge[-1] + 1):
            self.slot = k - edge[step]
            for unit in starts.get(k, ()):
                gen = unit()
                if gen is not None:
                    running.append([0, gen])
            for item in list(running):
                if item[0] <= k:
                    try:
                        item[0] = k + next(item[1])
                    except StopIteration:
                        running.remove(item)
            if step < len(steps) and k + 1 == edge[step + 1]:
                steps[step][0]()
                step += 1
        for item in running:
            for _ in item[1]:
                pass


def _kernel(x_hbm, wqkv_hbm, wo_hbm, w1_hbm, w2_hbm, o_hbm,
            stage, w1_v, w2_v,
            bq0_s, bq1_s, bk_s, bv_s, bo_s, b1_s, b2_s,
            ox_s, xb_s, ha_s, a2_s,
            q_s, k_s, v_s, p_s, st_s, h_s, out_s,
            xsem, qsem, wsem, fsem, osem):
    S, D = x_hbm.shape
    F = w2_hbm.shape[0]
    NT = S // TM
    NC = D // 128
    HC = NC // 2
    DQ, FQ = D // 4, F // 4
    NF = FQ // 128
    R1, R2 = w1_v.shape[0] - D, w2_v.shape[0] - F
    head_dim = D // HEADS
    oa_s, xa_s = ox_s.at[0], ox_s.at[1]
    sched = _Schedule()
    after, run = sched.after, sched.run

    def x_copy(k):
        rows = pl.ds(k * TM, TM if k < 4 else S - 4 * TM)
        return [pltpu.make_async_copy(x_hbm.at[rows], stage.at[rows], xsem.at[k])]

    def q_copy(g):
        rows = [_scaled(g + HC * half, 128) for half in range(2)]
        return [pltpu.make_async_copy(wqkv_hbm.at[pl.ds(r, 128), pl.ds(0, D)],
                                      stage.at[pl.ds(_aligned(S + r, 128), 128)], qsem.at[g]) for r in rows]

    def k_copy(g):
        rows = [pl.ds((2 * g + HC * half) * 128, 256) for half in range(2)]
        return [pltpu.make_async_copy(wqkv_hbm.at[r, pl.ds(D, D)], stage.at[pl.ds(S + D, D)].at[r], wsem.at[g])
                for r in rows]

    def w_copy(m):
        src = wo_hbm if m == 3 else wqkv_hbm.at[:, pl.ds(m * D, D)]
        return [pltpu.make_async_copy(src, stage.at[pl.ds(S + m * D, D)], wsem.at[m])]

    def f_copy(g):
        out = []
        for hbm, dst, blk, r in ((w1_hbm, w1_v, DQ, R1), (w2_hbm, w2_v, FQ, R2)):
            for q in range(4):
                rows = pl.ds(q * blk + 2 * r, blk - 2 * r) if g else pl.ds(q * blk, 2 * r)
                out.append(pltpu.make_async_copy(hbm.at[rows], dst.at[rows], fsem.at[g]))
        return out

    def o_copy(i, r0=0, nr=TM, c0=0, nc=D):
        return [pltpu.make_async_copy(out_s.at[i % 2, pl.ds(r0, nr), pl.ds(c0, nc)],
                                      o_hbm.at[pl.ds(_aligned(i * TM + r0, HM), nr), pl.ds(c0, nc)], osem.at[i % 2])]

    def scatter(dst, col, pair, blocks):
        f = []
        for q in range(4):
            f.append([_split(after(12, b)) for b in blocks[q]])
            yield 1
        for e in range(2):
            ops = [_rhs_ops(*[f[q][a][e] for q in range(4)]) for a in range(2)]
            for t in range(7):
                dst[t, col, pl.ds(16 * e + pair, 8, stride=GS), :] = _join(ops[0][t], ops[1][t])

    def prep_qkv(m, kt, dst, col, g):
        rows = [_aligned(S + m * D + (kt + HC * half) * 128, 128) for half in range(2)]
        tt = [pltpu.bitcast(stage[pl.ds(r, 128), g * 128:(g + 1) * 128].T, U32) for r in rows]
        yield 6
        for hp in range(2):
            yield from scatter(dst, col, 2 * g + hp,
                               [[tt[dr][32 * hp + 16 * a + 8 * dc:32 * hp + 16 * a + 8 * dc + 8] for a in range(2)]
                                for dr, dc in QUADS])

    def prep_o(pair, nt):
        def load(a, dr, dc):
            r, c = S + 3 * D + 64 * pair + 32 * a + 16 * dr, (nt + HC * dc) * 128
            return pltpu.bitcast(stage[r:r + 16, c:c + 128], U32)
        return scatter(bo_s, nt, pair, [[load(a, dr, dc) for a in range(2)] for dr, dc in QUADS])

    def two_levels(ops, fetch, pause, load, store):
        f = {}
        for qo, ts in fetch:
            f[qo] = {}
            for qi in (0, 3, 1, 2):
                f[qo][qi] = load(*_block_index(qo, qi))
                yield pause[len(ts) - 1]
            for t in ts:
                outer = [[ops(*[f[q][qi][e] if q in f else _Absent() for q in range(4)])[t] for qi in range(4)]
                         for e in range(2)]
                inner = [ops(*outer[e]) for e in range(2)]
                for u in range(7):
                    store(7 * t + u, _join(inner[0][u], inner[1][u]))

    def prep_ffn(src, dst, col, src_row, src_step, dst_row, r, n):
        def load(rb, cb):
            rows, c = pl.ds(_aligned(src_row + rb * src_step + r, 16), 16), col(cb, n) * 128
            return _split(after(12, pltpu.bitcast(src[rows, c:c + 128], U32)))

        def store(k, v):
            dst[n, k, pl.ds(_aligned(dst_row + r // 2, 8), 8), :] = v
        return two_levels(_rhs_ops, RHS_FETCH, (1, 1, 1), load, store)

    def prep_ffn_units(i):
        out = []
        for src, dst, blk, rows, chunks, col in ((w1_v, b1_s, DQ, R1, NF, lambda cb, n: cb * NF + n),
                                                 (w2_v, b2_s, FQ, R2, 2, lambda cb, n: 4 * n + cb)):
            if isinstance(i, int):
                r0 = (i - 2) * rows
                where, rows = (r0, blk, r0 // 2), blk - r0
            else:
                r0 = jnp.where(i > 1, (i - 2) * rows, 0)
                where = (jnp.where(i > 1, r0, 4 * blk), jnp.where(i > 1, blk, 0), r0 // 2)
            out.append([P(prep_ffn, src, dst, col, *where, r, n) for r in range(0, rows, 16) for n in range(chunks)])
        return out

    def permuted(ref, t, col, g0, groups):
        return jnp.concatenate([ref[t, col, GS * g:GS * g + 32, :] for g in range(g0, g0 + groups)], axis=0)

    def ln_stats(load, scale, pause, r):
        xs = [load(r, c) for c in range(NC)]
        xs = [[after(12, t[e]) if c == 0 else t[e] for c, t in enumerate(xs)] for e in range(2)]
        mu = [jnp.broadcast_to(jnp.sum(_tree(jnp.add, t), axis=-1, keepdims=True), (8, 128)) for t in xs]
        yield pause[0]
        mu = [after(12, m) * (1.0 / D) for m in mu]
        var = [_tree(jnp.add, [(t - m) * (t - m) for t in ts]) for ts, m in zip(xs, mu)]
        var = [jnp.broadcast_to(jnp.sum(v, axis=-1, keepdims=True), (8, 128)) for v in var]
        yield pause[1]
        for e in range(2):
            rs = lax.rsqrt(after(12, var[e]) * (1.0 / D) + EPS)
            st_s[0, r + 8 * e:r + 8 * e + 8, :] = mu[e]
            st_s[1, r + 8 * e:r + 8 * e + 8, :] = rs if scale == 1.0 else rs * scale

    def normalized(load, r, c):
        st = [[st_s[k, r + 8 * e:r + 8 * e + 8, :] for k in range(2)] for e in range(2)]
        return [(t - after(12, m)) * rs for t, (m, rs) in zip(load(r, c), st)]

    def ln_apply(load, dst, r, kt):
        ys = []
        for dr, dc in QUADS:
            ys.append(normalized(load, r + dr * HM, kt + dc * HC))
            yield 1
        ops = [_lhs_ops(*[y[e] for y in ys]) for e in range(2)]
        for t in range(7):
            dst[t, r // 2:r // 2 + 8, kt * 128:(kt + 1) * 128] = _join(ops[0][t], ops[1][t])

    def ln_apply2(load, r, n):
        def store(k, v):
            ha_s[k, r // 2:r // 2 + 8, n * 128:(n + 1) * 128] = v
        return two_levels(_lhs_ops, LHS_FETCH, (1, 2, 2),
                          lambda rb, cb: normalized(load, rb * QM + r, 2 * cb + n), store)

    def ln_x(i, dst):
        r0 = _scaled(i, TM)

        def load(r, c):
            return _split(pltpu.bitcast(stage[pl.ds(r0 + r, 16), c * 128:(c + 1) * 128], U32))
        return ([P(ln_stats, load, 1.0, (16, 16), r) for r in range(0, TM, 16)],
                [P(ln_apply, load, dst, r, kt) for kt in range(HC) for r in range(0, HM, 16)])

    def ln_h(i, pause):
        r0 = _scaled(i, TM)

        def load(r, c):
            return [h_s[c, pl.ds(r0 + r + e, 8, stride=2), :] for e in range(2)]
        return ([P(ln_stats, load, 0.5, pause, r) for r in range(0, TM, 16)],
                [P(ln_apply2, load, r, n) for n in range(2) for r in range(0, QM, 16)])

    def strassen(product, emit, k_tiles=HC):
        steps = []
        for n in range(HC):
            comb = _Combine(EARLY, P(emit, n))

            def step(t, n=n, comb=comb):
                sched.done.append((product(n, t), 2 * k_tiles))
                comb.push(sched.done[-1][0])
            steps += [(P(step, t), 2 * k_tiles) for t in EARLY]
        return steps

    def strassen2(chunks, k_tiles, product, emit, order, inner_order):
        steps = []
        for n in range(chunks):
            outer = [_Combine(order, P(emit, n, qi)) for qi in range(4)]
            inner = _Combine(inner_order, lambda qi, c, outer=outer: outer[qi].push(c))

            def step(k, n=n, inner=inner):
                sched.done.append((product(n, k), k_tiles))
                inner.push(sched.done[-1][0])
            steps += [(P(step, 7 * t + u), k_tiles) for t in order for u in inner_order]
        return steps

    wq_tiles = [((bq0_s, bq1_s)[kt // 2], kt % 2) for kt in range(HC)]
    wk_tiles, wv_tiles = ([(b_s, kt) for kt in range(HC)] for b_s in (bk_s, bv_s))

    def project(a_s, tiles, dst, row, k0=0, k1=HC):
        def product(n, t):
            rhs = jnp.concatenate([_bf16(permuted(b_s, t, col, 2 * n, 2)) for b_s, col in tiles[k0:k1]], axis=1)
            return lax.dot_general(_bf16(a_s[t, :, k0 * 128:k1 * 128]), rhs, NT_DIMS, preferred_element_type=F32)

        def emit(n, q, c):
            dr, dc = QUADS[q]
            at = (n + dc * HC, pl.ds(_aligned(row + dr * HM, 8), HM), slice(None))
            dst[at] = dst[at] + c if k0 else c
        return strassen(product, emit, k1 - k0)

    def out_project(i, a_s):
        r0 = _scaled(i, TM)

        def product(n, t):
            return jnp.dot(_bf16(a_s[t]), _bf16(permuted(bo_s, t, n, 0, NC)), preferred_element_type=F32)

        def emit(n, q, c):
            dr, dc = QUADS[q]
            rows, col = pl.ds(r0 + dr * HM, HM), n + dc * HC
            h_s[col, rows, :] = stage[rows, col * 128:(col + 1) * 128].astype(F32) + c
        return strassen(product, emit)

    row2 = 2 * lax.broadcasted_iota(jnp.int32, (8, 128), 0)

    def probs(first, r, e):
        pause = (0, 6, 4) if first else (2, 8, 6)
        qv = [q_s[c, pl.ds((0 if first else TM) + r + e, 8, stride=2), :] for c in range(NC)]
        ls = []
        for w in range(WINDOW):
            rows = pl.ds(HALO + r + e - DILATION * w, 8, stride=2)
            t = qv[0] * after(16, k_s[0, rows, :])
            for c in range(1, NC):
                t = t + qv[c] * k_s[c, rows, :]
            t = _tree(jnp.add, [t] + [pltpu.roll(t, HEADS * s, 1) for s in range(1, 128 // HEADS)])
            if first and r + e < DILATION * w:
                t = jnp.where(row2 + (r + e) >= DILATION * w, t, -1e9 * head_dim ** 0.5)
            ls.append(t)
            yield pause[0]
        mx = _tree(jnp.maximum, ls)
        yield pause[1]
        mx = after(16, mx)
        es = [jnp.exp2((t - mx) * (head_dim ** -0.5 * LOG2E)) for t in ls]
        total = _tree(jnp.add, es)
        yield pause[2]
        inv = 1.0 / after(16, total)
        for w in range(WINDOW):
            p_s[w, r + 8 * e:r + 8 * e + 8, :] = es[w] * inv

    def probs_units(first):
        return [P(probs, first, r, e) for r in range(0, TM, 16) for e in range(2)]

    def mix(dst, n, r):
        ops = []
        for e in range(2):
            blocks = []
            for rr in (r, r + HM):
                ps = [p_s[w, rr + 8 * e:rr + 8 * e + 8, :] for w in range(WINDOW)]
                for c in (n, n + HC):
                    acc = None
                    for w in range(WINDOW):
                        v = v_s[c, pl.ds(HALO + rr + e - DILATION * w, 8, stride=2), :]
                        acc = ps[w] * after(12, v) if w == 0 else acc + ps[w] * v
                    blocks.append(acc)
                    yield 1
            ops.append(_lhs_ops(*blocks))
        for t in range(7):
            dst[t, r // 2:r // 2 + 8, n * 128:(n + 1) * 128] = _join(ops[0][t], ops[1][t])

    def mix_units(dst):
        return [P(mix, dst, n, r) for n in range(HC) for r in range(0, HM, 16)]

    def shift_halo(ref):
        for c in range(NC):
            ref[c, 0:HALO, :] = ref[c, TM:TM + HALO, :]

    _start(x_copy(0) + x_copy(1) + sum(map(q_copy, range(HC)), []) + k_copy(0) + k_copy(1) + x_copy(2)
           + w_copy(2) + w_copy(3) + x_copy(3))
    for c in range(NC):
        k_s[c, 0:HALO, :] = jnp.zeros((HALO, 128), F32)
    w1_v[D:, :] = jnp.zeros((R1, F), BF16)
    w2_v[F:, :] = jnp.zeros((R2, D), BF16)
    _wait(x_copy(0))
    word = pltpu.bitcast(stage[0:16, 0:128], U32)
    sched.zero = (word * word) & 2
    _start(f_copy(0))

    def normalize_tile(i, carry):
        pl.when(i == 1)(P(_wait, x_copy(1)))
        for units in ln_x(i, ox_s.at[i]):
            run([], (units, 0, 0))
        return carry
    lax.fori_loop(0, 2, normalize_tile, 0)

    def prepare_q(kt, carry):
        _wait(q_copy(kt))
        run([], ([P(prep_qkv, 0, kt, bq0_s, kt, g) for g in range(NC)], 0, 0))
        return carry
    lax.fori_loop(0, HC // 2, prepare_q, 0)

    def first_half(i, carry):
        sched.done.clear()
        pl.when(i == 1)(P(_wait, q_copy(2) + q_copy(3)))
        run(project(ox_s.at[i], wq_tiles, q_s, i * TM, 0, HC // 2),
            ([P(prep_qkv, 0, 2 * i + kt, bq1_s, kt, g) for kt in range(2) for g in range(NC)], 2, 23))
        return carry
    lax.fori_loop(0, 2, first_half, 0)

    def second_half(i, carry):
        sched.done.clear()
        for g in range(2):
            pl.when(i == g)(P(_wait, k_copy(g)))
        run(project(ox_s.at[i], wq_tiles, q_s, i * TM, HC // 2, HC),
            ([P(prep_qkv, 1, 2 * i + kt, bk_s, 2 * i + kt, g) for kt in range(2) for g in range(NC)], 2, 23))
        return carry
    lax.fori_loop(0, 2, second_half, 0)

    sched.done.clear()
    _wait(x_copy(2))
    stats, apply = ln_x(2, xb_s)
    run(project(oa_s, wk_tiles, k_s, HALO) + project(oa_s, wv_tiles, v_s, HALO),
        (stats, 0, 6), (apply, 10, 17),
        ([P(_wait, w_copy(2)), P(_start, x_copy(4))], 17, 17),
        ([P(prep_qkv, 2, kt, bv_s, kt, g) for kt in range(HC) for g in range(NC)], 17, 27),
        (probs_units(True), 29, 47),
        ([P(_wait, w_copy(3)), P(_start, f_copy(1))], 47, 47),
        ([P(prep_o, pair, nt) for pair in range(HEADS // 2) for nt in range(HC)], 47, 56))
    for c in range(NC):
        v_s[c, 0:HALO, :] = jnp.broadcast_to(v_s[c, HALO:HALO + 1, :], (HALO, 128))

    def move(t, kt):
        xa_s[t, :, kt * 128:(kt + 1) * 128] = xb_s[t, :, kt * 128:(kt + 1) * 128]

    def attention(i, carry):
        sched.done.clear()
        for k, copies in ((1, x_copy(3)), (2, x_copy(4) + f_copy(0)), (4, f_copy(1))):
            pl.when(i == k)(P(_wait, copies))
        shift_halo(k_s)
        prep1, prep2 = prep_ffn_units(i)
        stats, apply = ln_x(jnp.minimum(i + 2, NT - 1), xb_s)
        run(project(xa_s, wk_tiles, k_s, HALO) + project(xa_s, wv_tiles, v_s, HALO) + project(xb_s, wq_tiles, q_s, TM)
            + out_project(i - 1, oa_s),
            (mix_units(oa_s), 1, 25), ([P(shift_halo, v_s)], 28, 28), (probs_units(False), 29, 58),
            ([P(move, t, kt) for t in EARLY for kt in range(HC)], 58, 80),
            (prep1, 58, 84), (prep2, 86, 108), (stats, 60, 82), (apply, 86, 110))
        return carry
    lax.fori_loop(1, NT - 1, attention, 0)

    sched.done.clear()
    shift_halo(k_s)
    prep1, prep2 = prep_ffn_units(NT - 1)
    stats, apply = ln_h(0, (16, 16))
    run(project(xa_s, wk_tiles, k_s, HALO) + project(xa_s, wv_tiles, v_s, HALO)
        + out_project(NT - 2, oa_s) + out_project(NT - 1, xb_s),
        (mix_units(oa_s), 1, 26), ([P(shift_halo, v_s)], 28, 28), (probs_units(False), 29, 56),
        (mix_units(xb_s), 60, 82), (prep1, 30, 80), (prep2, 80, 108), (stats, 84, 96), (apply, 98, 110))

    def feed_forward(i, carry):
        sched.done.clear()
        pl.when(i > 1)(lambda: _wait(o_copy(i - 2)))
        r0 = _scaled(i, TM)
        acts = {}

        def up(n, k):
            return jnp.dot(_bf16(ha_s[k]), _bf16(b1_s[n, k]), preferred_element_type=F32)

        def activate(n, qi, qo, y):
            acts[qo, qi] = y + y * jnp.tanh(y)
            if len(acts) == 16:
                outer = [_lhs_ops(*[acts[qo, qi] for qo in range(4)]) for qi in range(4)]
                for t in range(7):
                    for u, v in enumerate(_lhs_ops(*[outer[qi][t] for qi in range(4)])):
                        a2_s[7 * t + u, :, n * 128:(n + 1) * 128] = pltpu.bitcast(v.astype(BF16), U32)
                acts.clear()

        def down(n, k):
            return jnp.dot(_bf16(a2_s[k]), _bf16(b2_s[n, k]), preferred_element_type=F32)

        def finish(n, qi, qo, c):
            rb, cb = _block_index(qo, qi)
            col = 4 * n + cb
            out_s[i % 2, rb * QM:(rb + 1) * QM, col * 128:(col + 1) * 128] = (
                h_s[col, pl.ds(r0 + rb * QM, QM), :] + c).astype(BF16)

        stats, apply = ln_h(jnp.minimum(i + 1, NT - 1), (14, 15))
        last = 49 * (NF + 1)
        run(strassen2(NF, 2, up, activate, (4, 1, 3, 2, 0, 5, 6), (0, 1, 3, 2, 4, 5, 6))
            + strassen2(2, NF, down, finish, (0, 1, 2, 3, 4, 5, 6), (3, 1, 2, 5, 4, 0, 6)),
            (stats, last + 1, last + 11), (apply, last + 19, last + 45),
            ([P(_start, o_copy(i, 0, TM, 0, D // 2))], last, last),
            ([P(_start, o_copy(i, HM, HM, D // 2, D // 2) + o_copy(i, 0, HM, 3 * DQ, DQ))], last + 42, last + 42))
        _start(o_copy(i, 0, HM, D // 2, DQ))
        return carry
    lax.fori_loop(0, NT, feed_forward, 0)
    _wait(o_copy(NT - 2) + o_copy(NT - 1))


@jax.jit
def pallas_sequential_preLN__sliding_local_dilated__dense_activation_silu__prompt_kernel(
    A_x: jax.Array,
    A_wqkv: jax.Array,
    A_wo: jax.Array,
    B_x: jax.Array,
    B_w1: jax.Array,
    B_w2: jax.Array,
):
    del B_x
    B, S, D = A_x.shape
    F = B_w1.shape[1]
    assert (B, S, D, F) == (1, 2048, 1024, 3584)
    NC, slices = D // 128, S // TM - 2
    r1, r2 = (pl.cdiv(n // 4, 16 * slices) * 16 for n in (D, F))
    hbm = pl.BlockSpec(memory_space=pl.ANY)
    whole, half = (pltpu.VMEM((7, tiles, 8 * GS, 128), U32) for tiles in (NC // 2, NC // 4))
    out = pl.pallas_call(
        _kernel,
        in_specs=[hbm] * 5,
        out_specs=hbm,
        out_shape=jax.ShapeDtypeStruct((S, D), BF16),
        scratch_shapes=[
            pltpu.VMEM((S + 4 * D, D), BF16), pltpu.VMEM((D + r1, F), BF16), pltpu.VMEM((F + r2, D), BF16),
            half, half, whole, whole, whole,
            pltpu.VMEM((F // 512, 49, D // 8, 128), U32), pltpu.VMEM((D // 512, 49, F // 8, 128), U32),
            pltpu.VMEM((2, 7, HM // 2, D // 2), U32), pltpu.VMEM((7, HM // 2, D // 2), U32),
            pltpu.VMEM((49, QM // 2, D // 4), U32), pltpu.VMEM((49, QM // 2, F // 4), U32),
            pltpu.VMEM((NC, 2 * TM, 128), F32), pltpu.VMEM((NC, TM + HALO, 128), F32),
            pltpu.VMEM((NC, TM + HALO, 128), F32), pltpu.VMEM((WINDOW, TM, 128), F32),
            pltpu.VMEM((2, TM, 128), F32), pltpu.VMEM((NC, S, 128), F32), pltpu.VMEM((2, TM, D), BF16),
            pltpu.SemaphoreType.DMA((5,)), pltpu.SemaphoreType.DMA((NC // 2,)), pltpu.SemaphoreType.DMA((4,)),
            pltpu.SemaphoreType.DMA((2,)), pltpu.SemaphoreType.DMA((2,)),
        ],
        compiler_params=pltpu.CompilerParams(vmem_limit_bytes=124 * 1024 * 1024, disable_bounds_checks=True),
    )(A_x.reshape(S, D), A_wqkv, A_wo, B_w1, B_w2)
    return out.reshape(B, S, D)
```
